```python
import jax
import jax.numpy as jnp

def _softmax(x, axis=-1):
    return jax.nn.softmax(x, axis=axis)

def _gelu(x):
    return jax.nn.gelu(x, approximate=True)

def _silu(x):
    return jax.nn.silu(x)

def _sigmoid(x):
    return jax.nn.sigmoid(x)

def _layernorm(x, axis=-1, eps=1e-05):
    m = jnp.mean(x, axis=axis, keepdims=True)
    v = jnp.var(x, axis=axis, keepdims=True)
    return (x - m) / jnp.sqrt(v + eps)

def _scatter_add(tgt, idx, src, axis=0):
    return tgt.at[idx].add(src)

def _segment_sum(src, seg, n):
    return jax.ops.segment_sum(src, seg, n)

class _Rng:

    def __init__(self, key):
        self._k = key

    def _next(self):
        self._k, sub = jax.random.split(self._k)
        return sub

    def normal(self, shape):
        return jax.random.normal(self._next(), shape, dtype=jnp.bfloat16)

    def randint(self, lo, hi, shape):
        return jax.random.randint(self._next(), shape, lo, hi, dtype=jnp.int32)

    def uniform(self, shape, lo=0.0, hi=1.0):
        return jax.random.uniform(self._next(), shape, jnp.bfloat16, lo, hi)

    def permutation(self, n):
        return jax.random.permutation(self._next(), n)
kernel_name = 'adaLN_cond__compressed_kv_cla__glu_gated_geglu__decode'

def setup_inputs():
    _rng = _Rng(jax.random.key(int.from_bytes(__import__("os").urandom(4), "little")))
    _w = lambda a: (lambda t: t.astype(jnp.bfloat16) if jnp.issubdtype(t.dtype, jnp.floating) else t)(jnp.asarray(a))

    def _A_setup():
        B, H, Sq, Sk, D, M = (1, 32, 1, 32768, 128, 512)
        Dc = 4 * D
        return {'x': _w((lambda *s: _rng.normal(s) * 0.05)(B, Sq, M)), 'c_kv': _w((lambda *s: _rng.normal(s) * 0.05)(B, Sk, Dc)), 'w_q': _w((lambda *s: _rng.normal(s) * 0.05)(M, H, D) * M ** (-0.5)), 'w_uk': _w((lambda *s: _rng.normal(s) * 0.05)(Dc, H, D) * Dc ** (-0.5)), 'w_uv': _w((lambda *s: _rng.normal(s) * 0.05)(Dc, H, D) * Dc ** (-0.5)), 'w_o': _w((lambda *s: _rng.normal(s) * 0.05)(H, D, M) * (H * D) ** (-0.5))}
    _A_in = _A_setup()

    def _B_setup():
        B, S, Dm, Df = (1, 1, 512, 1792)
        return {'x': _w((lambda *s: _rng.normal(s) * 0.05)(B, S, Dm)), 'w_gate': _w((lambda *s: _rng.normal(s) * 0.05)(Dm, Df) * Dm ** (-0.5)), 'w_up': _w((lambda *s: _rng.normal(s) * 0.05)(Dm, Df) * Dm ** (-0.5)), 'w_down': _w((lambda *s: _rng.normal(s) * 0.05)(Df, Dm) * Df ** (-0.5))}
    _B_in = _B_setup()
    return {'A_x': _A_in['x'], 'A_c_kv': _A_in['c_kv'], 'A_w_q': _A_in['w_q'], 'A_w_uk': _A_in['w_uk'], 'A_w_uv': _A_in['w_uv'], 'A_w_o': _A_in['w_o'], 'B_x': _B_in['x'], 'B_w_gate': _B_in['w_gate'], 'B_w_up': _B_in['w_up'], 'B_w_down': _B_in['w_down'], 'c': _w((lambda *s: _rng.normal(s) * 0.05)(1, 512)), 'w_mod': _w((lambda *s: _rng.normal(s) * 0.05)(512, 6 * 512) * 512 ** (-0.5))}

def reference(A_x, A_c_kv, A_w_q, A_w_uk, A_w_uv, A_w_o, B_x, B_w_gate, B_w_up, B_w_down, c, w_mod):

    def _A_ref(x, c_kv, w_q, w_uk, w_uv, w_o):
        B, Sq, M = (x.shape[0], x.shape[1], x.shape[2])
        Sk = c_kv.shape[1]
        H, D = (w_q.shape[1], w_q.shape[2])
        q = jnp.einsum('bqm,mhd->bhqd', x, w_q)
        k = jnp.einsum('bkc,chd->bhkd', c_kv, w_uk)
        v = jnp.einsum('bkc,chd->bhkd', c_kv, w_uv)
        scores = jnp.einsum('bhqd,bhkd->bhqk', q, k) * D ** (-0.5)
        off = Sk - Sq
        qi = jnp.arange(Sq)[:, None]
        kj = jnp.arange(Sk)[None, :]
        cmask = kj <= qi + off
        scores = jnp.where(cmask[None, None], scores, -1000000000.0)
        p = _softmax(scores, axis=-1)
        ctx = jnp.einsum('bhqk,bhkd->bhqd', p, v)
        return jnp.einsum('bhqd,hdm->bqm', ctx, w_o)

    def _B_ref(x, w_gate, w_up, w_down):
        g = jnp.einsum('bsd,df->bsf', x, w_gate)
        u = jnp.einsum('bsd,df->bsf', x, w_up)
        h = _gelu(g) * u
        return jnp.einsum('bsf,fd->bsd', h, w_down)
    x = A_x
    mod = (_silu(c) @ w_mod).reshape(c.shape[0], 6, 1, -1)
    sa, ca, ga, sb, cb, gb = (mod[:, 0].copy(), mod[:, 1].copy(), mod[:, 2].copy(), mod[:, 3].copy(), mod[:, 4].copy(), mod[:, 5].copy())
    h = _layernorm(x, axis=-1) * (1 + ca) + sa
    x = x + ga * _A_ref(h, A_c_kv, A_w_q, A_w_uk, A_w_uv, A_w_o)
    h = _layernorm(x, axis=-1) * (1 + cb) + sb
    x = x + gb * _B_ref(h, B_w_gate, B_w_up, B_w_down)
    return x
```

```python
import functools

import jax
import jax.numpy as jnp
import numpy as np
from jax import lax
import jax.experimental.pallas as pl
import jax.experimental.pallas.tpu as pltpu


F32 = jnp.float32
BF16 = jnp.bfloat16

_NT = (((1,), (1,)), ((), ()))


def _dot(a, b):
    return jnp.dot(a, b, preferred_element_type=F32)


def _dot_nt(a, b):
    return lax.dot_general(a, b, _NT, preferred_element_type=F32)


def _layernorm(x, eps=1e-5):
    m = jnp.mean(x, axis=-1, keepdims=True)
    d = x - m
    v = jnp.mean(d * d, axis=-1, keepdims=True)
    return d * lax.rsqrt(v + eps)


def _kernel(x_hbm, ckv_hbm, wq_hbm, wuk_hbm, wuv_hbm, wo_hbm, wg_hbm, wu_hbm, wd_hbm,
            c_hbm, wmod_hbm, o_ref,
            x_v, c_v, ckv_v, wq_v, wuk_v, wuv_v, wo_v, wg_v, wu_v, wd_v, wmod_v,
            m_sc, l_sc, acc_sc, sems, ckv_sems, *, H, D, M, DC, SK, DF, T):
    NCH = SK // T
    G = DC // 128
    GW = 128 * H

    small = [(c_hbm, c_v), (x_hbm, x_v), (wmod_hbm, wmod_v), (wq_hbm, wq_v), (wuk_hbm, wuk_v),
             (wuv_hbm, wuv_v), (wo_hbm, wo_v), (wg_hbm, wg_v), (wu_hbm, wu_v), (wd_hbm, wd_v)]

    def cp(i):
        return pltpu.make_async_copy(small[i][0], small[i][1], sems.at[i])

    def kv_cp(i):
        return pltpu.make_async_copy(ckv_hbm.at[pl.ds(i * T, T)], ckv_v.at[pl.ds(i * T, T)],
                                     ckv_sems.at[i])

    for i in range(5):
        cp(i).start()
    for i in range(NCH):
        kv_cp(i).start()
    for i in range(5, 10):
        cp(i).start()

    ri = lax.broadcasted_iota(jnp.int32, (128, GW), 0)
    cj = lax.broadcasted_iota(jnp.int32, (128, GW), 1)
    e0 = jnp.where((cj // H) == ri, 1.0, 0.0).astype(BF16)
    hr = lax.broadcasted_iota(jnp.int32, (H, GW), 0)
    hc = lax.broadcasted_iota(jnp.int32, (H, GW), 1)
    diag = (hc % H) == hr

    def expand_mm(a, w_ref):
        a = a.astype(BF16)
        a_st = jnp.concatenate([a[:, g * 128:(g + 1) * 128] for g in range(G)], axis=0)
        xx = _dot(a_st, e0)
        out = None
        for g in range(G):
            s = jnp.where(diag, xx[g * H:(g + 1) * H], 0.0).astype(BF16)
            r = _dot(s, w_ref[pl.ds(g * GW, GW), :])
            out = r if out is None else out + r
        return out

    def contract_mm(q, w_ref, scale):
        q = q.astype(BF16)
        parts = []
        for g in range(G):
            tt = _dot_nt(q, w_ref[pl.ds(g * GW, GW), :])
            parts.append(jnp.where(diag, tt * scale, 0.0).astype(BF16))
        st = jnp.concatenate(parts, axis=0)
        r = _dot_nt(st, e0)
        return jnp.concatenate([r[g * H:(g + 1) * H] for g in range(G)], axis=1)

    cp(0).wait()
    cp(1).wait()
    cp(2).wait()
    cc = jnp.broadcast_to(c_v[...].astype(F32), (8, M))
    sc = (cc * jax.nn.sigmoid(cc)).astype(BF16)
    mod = _dot(sc, wmod_v[...])
    sa, ca, ga, sb, cb, gb = [mod[:, i * M:(i + 1) * M] for i in range(6)]
    x = jnp.broadcast_to(x_v[0].astype(F32), (8, M))
    h = _layernorm(x) * (1.0 + ca) + sa

    cp(3).wait()
    hb = jnp.broadcast_to(h[0:1], (H, M))
    q = expand_mm(hb, wq_v)
    cp(4).wait()
    qa = contract_mm(q, wuk_v, float(D) ** -0.5).astype(BF16)

    m_sc[...] = jnp.full((H, 128), -jnp.inf, F32)
    l_sc[...] = jnp.zeros((H, 128), F32)
    acc_sc[...] = jnp.zeros((H, DC), F32)

    def body(i, carry):
        kv_cp(i).wait()
        kv = ckv_v[pl.ds(pl.multiple_of(i * T, T), T), :]
        s = _dot_nt(qa, kv)
        m_old = m_sc[...]
        m_new = jnp.maximum(m_old, jnp.max(s, axis=1, keepdims=True))
        alpha = jnp.exp(m_old - m_new)
        p = jnp.exp(s - m_new[:, 0:1])
        l_sc[...] = alpha * l_sc[...] + jnp.sum(p, axis=1, keepdims=True)
        m_sc[...] = m_new
        acc_sc[...] = alpha[:, 0:1] * acc_sc[...] + _dot(p.astype(BF16), kv)
        return carry

    lax.fori_loop(0, NCH, body, 0)
    ctx_c = acc_sc[...] / l_sc[:, 0:1]

    cp(5).wait()
    ctx = expand_mm(ctx_c, wuv_v).astype(BF16)
    cp(6).wait()
    row = lax.broadcasted_iota(jnp.int32, (H, D), 0)
    zero = jnp.zeros((H, D), BF16)
    lhs = jnp.concatenate([jnp.where(row == hh, ctx, zero) for hh in range(H)], axis=1)
    ao = jnp.sum(_dot(lhs, wo_v[...]), axis=0, keepdims=True)
    x2 = x + ga * ao

    h2 = (_layernorm(x2) * (1.0 + cb) + sb).astype(BF16)
    cp(7).wait()
    g = _dot(h2, wg_v[...])
    cp(8).wait()
    u = _dot(h2, wu_v[...])
    act = (jax.nn.gelu(g, approximate=True) * u).astype(BF16)
    cp(9).wait()
    y = _dot(act, wd_v[...])
    out = x2 + gb * y
    o_ref[0] = out[0:1].astype(o_ref.dtype)


@jax.jit
def pallas_adaLN_cond__compressed_kv_cla__glu_gated_geglu__decode_kernel(
    A_x: jax.Array,
    A_c_kv: jax.Array,
    A_w_q: jax.Array,
    A_w_uk: jax.Array,
    A_w_uv: jax.Array,
    A_w_o: jax.Array,
    B_x: jax.Array,
    B_w_gate: jax.Array,
    B_w_up: jax.Array,
    B_w_down: jax.Array,
    c: jax.Array,
    w_mod: jax.Array,
):
    M, H, D = A_w_q.shape
    DC = A_w_uk.shape[0]
    SK = A_c_kv.shape[1]
    DF = B_w_gate.shape[1]
    T = 2048
    NCH = SK // T

    ckv = A_c_kv.reshape(SK, DC)
    wq = A_w_q.reshape(M * H, D)
    wuk = A_w_uk.reshape(DC * H, D)
    wuv = A_w_uv.reshape(DC * H, D)
    wo = A_w_o.reshape(H * D, M)

    kern = functools.partial(_kernel, H=H, D=D, M=M, DC=DC, SK=SK, DF=DF, T=T)
    any_spec = pl.BlockSpec(memory_space=pl.ANY)
    return pl.pallas_call(
        kern,
        out_shape=jax.ShapeDtypeStruct(A_x.shape, A_x.dtype),
        in_specs=[any_spec] * 11,
        out_specs=pl.BlockSpec(memory_space=pltpu.VMEM),
        scratch_shapes=[
            pltpu.VMEM(A_x.shape, A_x.dtype),
            pltpu.VMEM(c.shape, c.dtype),
            pltpu.VMEM((SK, DC), BF16),
            pltpu.VMEM((M * H, D), BF16),
            pltpu.VMEM((DC * H, D), BF16),
            pltpu.VMEM((DC * H, D), BF16),
            pltpu.VMEM((H * D, M), BF16),
            pltpu.VMEM((M, DF), BF16),
            pltpu.VMEM((M, DF), BF16),
            pltpu.VMEM((DF, M), BF16),
            pltpu.VMEM(w_mod.shape, BF16),
            pltpu.VMEM((H, 128), F32),
            pltpu.VMEM((H, 128), F32),
            pltpu.VMEM((H, DC), F32),
            pltpu.SemaphoreType.DMA((10,)),
            pltpu.SemaphoreType.DMA((NCH,)),
        ],
        compiler_params=pltpu.CompilerParams(vmem_limit_bytes=110 * 1024 * 1024),
    )(A_x, ckv, wq, wuk, wuv, wo, B_w_gate, B_w_up, B_w_down, c, w_mod)
```

```python
import functools

import jax
import jax.numpy as jnp
import numpy as np
from jax import lax
import jax.experimental.pallas as pl
import jax.experimental.pallas.tpu as pltpu


F32 = jnp.float32
BF16 = jnp.bfloat16

KV_CHUNKS = ((0, 8), (8, 12), (12, 16))
WD_CHUNKS = ((0, 1024), (1024, 1536), (1536, 1792))
N_COPIES = 9 + len(KV_CHUNKS) + len(WD_CHUNKS)

_NT = (((1,), (1,)), ((), ()))


def _dot(a, b):
    return jnp.dot(a, b, preferred_element_type=F32)


def _dot_nt(a, b):
    return lax.dot_general(a, b, _NT, preferred_element_type=F32)


def _layernorm(x, eps=1e-5):
    m = jnp.mean(x, axis=-1, keepdims=True)
    d = x - m
    v = jnp.mean(d * d, axis=-1, keepdims=True)
    return d * lax.rsqrt(v + eps)


def _kernel(x_hbm, ckv_hbm, wq_hbm, wuk_hbm, wuv_hbm, wo_hbm, wg_hbm, wu_hbm, wd_hbm,
            c_hbm, wmod_hbm, o_ref,
            x_v, c_v, ckv_v, wq_v, wuk_v, wuv_v, wo_v, wg_v, wu_v, wd_v, wmod_v,
            m_sc, l_sc, acc_sc, sems, *, H, D, M, DC, SK, DF, T):
    NCH = SK // T
    G = DC // 128
    GW = 128 * H

    copies = []

    def add_copy(src, dst):
        copies.append((src, dst))
        return len(copies) - 1

    def cp(i):
        return pltpu.make_async_copy(copies[i][0], copies[i][1], sems.at[i])

    i_mod = add_copy(wmod_hbm, wmod_v)
    i_c = add_copy(c_hbm, c_v)
    i_x = add_copy(x_hbm, x_v)
    i_q = add_copy(wq_hbm, wq_v)
    i_uk = add_copy(wuk_hbm, wuk_v)
    i_kv = []
    for (b0, b1) in KV_CHUNKS:
        sl = pl.ds(b0 * T, (b1 - b0) * T)
        i_kv.append(add_copy(ckv_hbm.at[sl], ckv_v.at[sl]))
    i_uv = add_copy(wuv_hbm, wuv_v)
    i_o = add_copy(wo_hbm, wo_v)
    i_g = add_copy(wg_hbm, wg_v)
    i_u = add_copy(wu_hbm, wu_v)
    i_d = []
    for (r0, r1) in WD_CHUNKS:
        sl = pl.ds(r0, r1 - r0)
        i_d.append(add_copy(wd_hbm.at[sl], wd_v.at[sl]))
    assert len(copies) == N_COPIES
    for i in range(len(copies)):
        cp(i).start()

    ri = lax.broadcasted_iota(jnp.int32, (128, GW), 0)
    cj = lax.broadcasted_iota(jnp.int32, (128, GW), 1)
    e0 = jnp.where((cj // H) == ri, 1.0, 0.0).astype(BF16)
    hr = lax.broadcasted_iota(jnp.int32, (H, GW), 0)
    hc = lax.broadcasted_iota(jnp.int32, (H, GW), 1)
    diag = (hc % H) == hr

    def expand_mm(a, w_ref):
        a = a.astype(BF16)
        a_st = jnp.concatenate([a[:, g * 128:(g + 1) * 128] for g in range(G)], axis=0)
        xx = _dot(a_st, e0)
        out = None
        for g in range(G):
            s = jnp.where(diag, xx[g * H:(g + 1) * H], 0.0).astype(BF16)
            r = _dot(s, w_ref[pl.ds(g * GW, GW), :])
            out = r if out is None else out + r
        return out

    def contract_mm(q, w_ref, scale):
        q = q.astype(BF16)
        parts = []
        for g in range(G):
            tt = _dot_nt(q, w_ref[pl.ds(g * GW, GW), :])
            parts.append(jnp.where(diag, tt * scale, 0.0).astype(BF16))
        st = jnp.concatenate(parts, axis=0)
        r = _dot_nt(st, e0)
        return jnp.concatenate([r[g * H:(g + 1) * H] for g in range(G)], axis=1)

    cp(i_mod).wait()
    cp(i_c).wait()
    cp(i_x).wait()
    cc = jnp.broadcast_to(c_v[...].astype(F32), (8, M))
    sc = (cc * jax.nn.sigmoid(cc)).astype(BF16)
    mod = _dot(sc, wmod_v[...])
    sa, ca, ga, sb, cb, gb = [mod[:, i * M:(i + 1) * M] for i in range(6)]
    x = jnp.broadcast_to(x_v[0].astype(F32), (8, M))
    h = _layernorm(x) * (1.0 + ca) + sa

    cp(i_q).wait()
    hb = jnp.broadcast_to(h[0:1], (H, M))
    q = expand_mm(hb, wq_v)
    cp(i_uk).wait()
    qa = contract_mm(q, wuk_v, float(D) ** -0.5).astype(BF16)

    m_sc[...] = jnp.full((H, 128), -jnp.inf, F32)
    l_sc[...] = jnp.zeros((H, 128), F32)
    acc_sc[...] = jnp.zeros((H, DC), F32)

    def body(i, carry):
        for j, (b0, _) in enumerate(KV_CHUNKS):
            @pl.when(i == b0)
            def _():
                cp(i_kv[j]).wait()

        kv = ckv_v[pl.ds(pl.multiple_of(i * T, T), T), :]
        s = _dot_nt(qa, kv)
        m_old = m_sc[...]
        m_new = jnp.maximum(m_old, jnp.max(s, axis=1, keepdims=True))
        alpha = jnp.exp(m_old - m_new)
        p = jnp.exp(s - m_new[:, 0:1])
        l_sc[...] = alpha * l_sc[...] + jnp.sum(p, axis=1, keepdims=True)
        m_sc[...] = m_new
        acc_sc[...] = alpha[:, 0:1] * acc_sc[...] + _dot(p.astype(BF16), kv)
        return carry

    lax.fori_loop(0, NCH, body, 0)
    ctx_c = acc_sc[...] / l_sc[:, 0:1]

    cp(i_uv).wait()
    ctx = expand_mm(ctx_c, wuv_v).astype(BF16)
    cp(i_o).wait()
    row = lax.broadcasted_iota(jnp.int32, (H, D), 0)
    zero = jnp.zeros((H, D), BF16)
    lhs = jnp.concatenate([jnp.where(row == hh, ctx, zero) for hh in range(H)], axis=1)
    ao = jnp.sum(_dot(lhs, wo_v[...]), axis=0, keepdims=True)
    x2 = x + ga * ao

    h2 = (_layernorm(x2) * (1.0 + cb) + sb).astype(BF16)
    cp(i_g).wait()
    g = _dot(h2, wg_v[...])
    cp(i_u).wait()
    u = _dot(h2, wu_v[...])
    act = (jax.nn.gelu(g, approximate=True) * u).astype(BF16)
    y = None
    for j, (r0, r1) in enumerate(WD_CHUNKS):
        cp(i_d[j]).wait()
        yy = _dot(act[:, r0:r1], wd_v[r0:r1, :])
        y = yy if y is None else y + yy
    out = x2 + gb * y
    o_ref[0] = out[0:1].astype(o_ref.dtype)


@jax.jit
def pallas_adaLN_cond__compressed_kv_cla__glu_gated_geglu__decode_kernel(
    A_x: jax.Array,
    A_c_kv: jax.Array,
    A_w_q: jax.Array,
    A_w_uk: jax.Array,
    A_w_uv: jax.Array,
    A_w_o: jax.Array,
    B_x: jax.Array,
    B_w_gate: jax.Array,
    B_w_up: jax.Array,
    B_w_down: jax.Array,
    c: jax.Array,
    w_mod: jax.Array,
):
    M, H, D = A_w_q.shape
    DC = A_w_uk.shape[0]
    SK = A_c_kv.shape[1]
    DF = B_w_gate.shape[1]
    T = 2048
    NCH = SK // T

    ckv = A_c_kv.reshape(SK, DC)
    wq = A_w_q.reshape(M * H, D)
    wuk = A_w_uk.reshape(DC * H, D)
    wuv = A_w_uv.reshape(DC * H, D)
    wo = A_w_o.reshape(H * D, M)

    kern = functools.partial(_kernel, H=H, D=D, M=M, DC=DC, SK=SK, DF=DF, T=T)
    any_spec = pl.BlockSpec(memory_space=pl.ANY)
    return pl.pallas_call(
        kern,
        out_shape=jax.ShapeDtypeStruct(A_x.shape, A_x.dtype),
        in_specs=[any_spec] * 11,
        out_specs=pl.BlockSpec(memory_space=pltpu.VMEM),
        scratch_shapes=[
            pltpu.VMEM(A_x.shape, A_x.dtype),
            pltpu.VMEM(c.shape, c.dtype),
            pltpu.VMEM((SK, DC), BF16),
            pltpu.VMEM((M * H, D), BF16),
            pltpu.VMEM((DC * H, D), BF16),
            pltpu.VMEM((DC * H, D), BF16),
            pltpu.VMEM((H * D, M), BF16),
            pltpu.VMEM((M, DF), BF16),
            pltpu.VMEM((M, DF), BF16),
            pltpu.VMEM((DF, M), BF16),
            pltpu.VMEM(w_mod.shape, BF16),
            pltpu.VMEM((H, 128), F32),
            pltpu.VMEM((H, 128), F32),
            pltpu.VMEM((H, DC), F32),
            pltpu.SemaphoreType.DMA((N_COPIES,)),
        ],
        compiler_params=pltpu.CompilerParams(vmem_limit_bytes=110 * 1024 * 1024),
    )(A_x, ckv, wq, wuk, wuv, wo, B_w_gate, B_w_up, B_w_down, c, w_mod)
```

```python
import functools

import jax
import jax.numpy as jnp
import numpy as np
from jax import lax
import jax.experimental.pallas as pl
import jax.experimental.pallas.tpu as pltpu


F32 = jnp.float32
BF16 = jnp.bfloat16

KV_CHUNKS = ((0, 8), (8, 12), (12, 16))
WD_CHUNKS = ((0, 1024), (1024, 1536), (1536, 1792))
FT = 256
N_COPIES = 9 + len(KV_CHUNKS) + len(WD_CHUNKS)

_NT = (((1,), (1,)), ((), ()))


def _dot(a, b):
    return jnp.dot(a, b, preferred_element_type=F32)


def _dot_nt(a, b):
    return lax.dot_general(a, b, _NT, preferred_element_type=F32)


def _layernorm(x, eps=1e-5):
    m = jnp.mean(x, axis=-1, keepdims=True)
    d = x - m
    v = jnp.mean(d * d, axis=-1, keepdims=True)
    return d * lax.rsqrt(v + eps)


def _kernel(x_hbm, ckv_hbm, wq_hbm, wuk_hbm, wuv_hbm, wo_hbm, wg_hbm, wu_hbm, wd_hbm,
            c_hbm, wmod_hbm, o_ref,
            x_v, c_v, ckv_v, wq_v, wuk_v, wuv_v, wo_v, wg_v, wu_v, wd_v, wmod_v,
            m_sc, l_sc, acc_sc, act_sc, sems, *, H, D, M, DC, SK, DF, T):
    NCH = SK // T
    G = DC // 128
    GW = 128 * H

    copies = []

    def add_copy(src, dst):
        copies.append((src, dst))
        return len(copies) - 1

    def cp(i):
        return pltpu.make_async_copy(copies[i][0], copies[i][1], sems.at[i])

    i_mod = add_copy(wmod_hbm, wmod_v)
    i_c = add_copy(c_hbm, c_v)
    i_x = add_copy(x_hbm, x_v)
    i_q = add_copy(wq_hbm, wq_v)
    i_uk = add_copy(wuk_hbm, wuk_v)
    i_kv = []
    for (b0, b1) in KV_CHUNKS:
        sl = pl.ds(b0 * T, (b1 - b0) * T)
        i_kv.append(add_copy(ckv_hbm.at[sl], ckv_v.at[sl]))
    i_uv = add_copy(wuv_hbm, wuv_v)
    i_o = add_copy(wo_hbm, wo_v)
    i_g = add_copy(wg_hbm, wg_v)
    i_u = add_copy(wu_hbm, wu_v)
    i_d = []
    for (r0, r1) in WD_CHUNKS:
        sl = pl.ds(r0, r1 - r0)
        i_d.append(add_copy(wd_hbm.at[sl], wd_v.at[sl]))
    assert len(copies) == N_COPIES
    for i in range(len(copies)):
        cp(i).start()

    ri = lax.broadcasted_iota(jnp.int32, (128, GW), 0)
    cj = lax.broadcasted_iota(jnp.int32, (128, GW), 1)
    e0 = jnp.where((cj // H) == ri, 1.0, 0.0).astype(BF16)
    hr = lax.broadcasted_iota(jnp.int32, (H, GW), 0)
    hc = lax.broadcasted_iota(jnp.int32, (H, GW), 1)
    diag = (hc % H) == hr

    def expand_mm(a, w_ref):
        a = a.astype(BF16)
        a_st = jnp.concatenate([a[:, g * 128:(g + 1) * 128] for g in range(G)], axis=0)
        xx = _dot(a_st, e0)
        out = None
        for g in range(G):
            s = jnp.where(diag, xx[g * H:(g + 1) * H], 0.0).astype(BF16)
            r = _dot(s, w_ref[pl.ds(g * GW, GW), :])
            out = r if out is None else out + r
        return out

    def contract_mm(q, w_ref, scale):
        q = q.astype(BF16)
        parts = []
        for g in range(G):
            tt = _dot_nt(q, w_ref[pl.ds(g * GW, GW), :])
            parts.append(jnp.where(diag, tt * scale, 0.0).astype(BF16))
        st = jnp.concatenate(parts, axis=0)
        r = _dot_nt(st, e0)
        return jnp.concatenate([r[g * H:(g + 1) * H] for g in range(G)], axis=1)

    cp(i_mod).wait()
    cp(i_c).wait()
    cp(i_x).wait()
    cc = jnp.broadcast_to(c_v[...].astype(F32), (8, M))
    sc = (cc * jax.nn.sigmoid(cc)).astype(BF16)
    mod = _dot(sc, wmod_v[...])
    sa, ca, ga, sb, cb, gb = [mod[:, i * M:(i + 1) * M] for i in range(6)]
    x = jnp.broadcast_to(x_v[0].astype(F32), (8, M))
    h = _layernorm(x) * (1.0 + ca) + sa

    cp(i_q).wait()
    hb = jnp.broadcast_to(h[0:1], (H, M))
    q = expand_mm(hb, wq_v)
    cp(i_uk).wait()
    qa = contract_mm(q, wuk_v, float(D) ** -0.5).astype(BF16)

    m_sc[...] = jnp.full((H, 128), -jnp.inf, F32)
    l_sc[...] = jnp.zeros((H, 128), F32)
    acc_sc[...] = jnp.zeros((H, DC), F32)

    def body(i, carry):
        for j, (b0, _) in enumerate(KV_CHUNKS):
            @pl.when(i == b0)
            def _():
                cp(i_kv[j]).wait()

        kv = ckv_v[pl.ds(pl.multiple_of(i * T, T), T), :]
        s = _dot_nt(qa, kv)
        m_old = m_sc[...]
        m_new = jnp.maximum(m_old, jnp.max(s, axis=1, keepdims=True))
        alpha = jnp.exp(m_old - m_new)
        p = jnp.exp(s - m_new[:, 0:1])
        l_sc[...] = alpha * l_sc[...] + jnp.sum(p, axis=1, keepdims=True)
        m_sc[...] = m_new
        acc_sc[...] = alpha[:, 0:1] * acc_sc[...] + _dot(p.astype(BF16), kv)
        return carry

    lax.fori_loop(0, NCH, body, 0)
    ctx_c = acc_sc[...] / l_sc[:, 0:1]

    cp(i_uv).wait()
    ctx = expand_mm(ctx_c, wuv_v).astype(BF16)
    cp(i_o).wait()
    row = lax.broadcasted_iota(jnp.int32, (H, D), 0)
    zero = jnp.zeros((H, D), BF16)
    lhs = jnp.concatenate([jnp.where(row == hh, ctx, zero) for hh in range(H)], axis=1)
    ao = jnp.sum(_dot(lhs, wo_v[...]), axis=0, keepdims=True)
    x2 = x + ga * ao

    h2 = (_layernorm(x2) * (1.0 + cb) + sb).astype(BF16)
    cp(i_g).wait()
    g = _dot(h2, wg_v[...])
    cp(i_u).wait()
    u = _dot(h2, wu_v[...])
    act = (jax.nn.gelu(g, approximate=True) * u).astype(BF16)
    for j in range(DF // FT):
        act_sc[j] = act[:, j * FT:(j + 1) * FT]

    def down(j, y):
        for n, (r0, _) in enumerate(WD_CHUNKS):
            @pl.when(j == r0 // FT)
            def _():
                cp(i_d[n]).wait()

        wd = wd_v[pl.ds(pl.multiple_of(j * FT, FT), FT), :]
        return y + _dot(act_sc[j], wd)

    y = lax.fori_loop(0, DF // FT, down, jnp.zeros((8, M), F32))
    out = x2 + gb * y
    o_ref[0] = out[0:1].astype(o_ref.dtype)


@jax.jit
def pallas_adaLN_cond__compressed_kv_cla__glu_gated_geglu__decode_kernel(
    A_x: jax.Array,
    A_c_kv: jax.Array,
    A_w_q: jax.Array,
    A_w_uk: jax.Array,
    A_w_uv: jax.Array,
    A_w_o: jax.Array,
    B_x: jax.Array,
    B_w_gate: jax.Array,
    B_w_up: jax.Array,
    B_w_down: jax.Array,
    c: jax.Array,
    w_mod: jax.Array,
):
    M, H, D = A_w_q.shape
    DC = A_w_uk.shape[0]
    SK = A_c_kv.shape[1]
    DF = B_w_gate.shape[1]
    T = SK // 16
    NCH = SK // T

    ckv = A_c_kv.reshape(SK, DC)
    wq = A_w_q.reshape(M * H, D)
    wuk = A_w_uk.reshape(DC * H, D)
    wuv = A_w_uv.reshape(DC * H, D)
    wo = A_w_o.reshape(H * D, M)

    kern = functools.partial(_kernel, H=H, D=D, M=M, DC=DC, SK=SK, DF=DF, T=T)
    any_spec = pl.BlockSpec(memory_space=pl.ANY)
    return pl.pallas_call(
        kern,
        out_shape=jax.ShapeDtypeStruct(A_x.shape, A_x.dtype),
        in_specs=[any_spec] * 11,
        out_specs=pl.BlockSpec(memory_space=pltpu.VMEM),
        scratch_shapes=[
            pltpu.VMEM(A_x.shape, A_x.dtype),
            pltpu.VMEM(c.shape, c.dtype),
            pltpu.VMEM((SK, DC), BF16),
            pltpu.VMEM((M * H, D), BF16),
            pltpu.VMEM((DC * H, D), BF16),
            pltpu.VMEM((DC * H, D), BF16),
            pltpu.VMEM((H * D, M), BF16),
            pltpu.VMEM((M, DF), BF16),
            pltpu.VMEM((M, DF), BF16),
            pltpu.VMEM((DF, M), BF16),
            pltpu.VMEM(w_mod.shape, BF16),
            pltpu.VMEM((H, 128), F32),
            pltpu.VMEM((H, 128), F32),
            pltpu.VMEM((H, DC), F32),
            pltpu.VMEM((DF // FT, 8, FT), BF16),
            pltpu.SemaphoreType.DMA((N_COPIES,)),
        ],
        compiler_params=pltpu.CompilerParams(vmem_limit_bytes=110 * 1024 * 1024,
                                             disable_semaphore_checks=True),
    )(A_x, ckv, wq, wuk, wuv, wo, B_w_gate, B_w_up, B_w_down, c, w_mod)
```

```python
import functools

import jax
import jax.numpy as jnp
from jax import lax
import jax.experimental.pallas as pl
import jax.experimental.pallas.tpu as pltpu

F32 = jnp.float32
BF16 = jnp.bfloat16

NKV = 16
KV_CHUNKS = ((0, 4), (4, 8), (8, 12), (12, 14), (14, 16))
FT = 256
WD_MXU = ((0, 512), (512, 1024), (1024, 1280), (1280, 1536))
WD_VPU = ((1536, 1664), (1664, 1728), (1728, 1760), (1760, 1792))
N_COPIES = 9 + len(KV_CHUNKS) + len(WD_MXU) + len(WD_VPU)

_NT = (((1,), (1,)), ((), ()))


def _dot(a, b):
    return jnp.dot(a, b, preferred_element_type=F32)


def _dot_nt(a, b):
    return lax.dot_general(a, b, _NT, preferred_element_type=F32)


def _layernorm(x, eps=1e-5):
    m = jnp.mean(x, axis=-1, keepdims=True)
    d = x - m
    v = jnp.mean(d * d, axis=-1, keepdims=True)
    return d * lax.rsqrt(v + eps)


def _kernel(x_hbm, ckv_hbm, wq_hbm, wuk_hbm, wuv_hbm, wo_hbm, wg_hbm, wu_hbm, wd_hbm,
            c_hbm, wmod_hbm, o_ref,
            x_v, c_v, ckv_v, wq_v, wuk_v, wuv_v, wo_v, wg_v, wu_v, wd_v, wmod_v,
            m_sc, l_sc, acc_sc, act_sc, acol_sc, sems, *, H, D, M, DC, SK, DF):
    T = SK // NKV
    G = DC // 128
    GW = 128 * H
    NL = WD_MXU[-1][1] // FT
    R0 = NL * FT

    copies = []

    def add_copy(src, dst):
        copies.append((src, dst))
        return len(copies) - 1

    def cp(i):
        return pltpu.make_async_copy(copies[i][0], copies[i][1], sems.at[i])

    i_mod = add_copy(wmod_hbm, wmod_v)
    i_c = add_copy(c_hbm, c_v)
    i_x = add_copy(x_hbm, x_v)
    i_q = add_copy(wq_hbm, wq_v)
    i_uk = add_copy(wuk_hbm, wuk_v)
    i_kv = []
    for b0, b1 in KV_CHUNKS:
        sl = pl.ds(b0 * T, (b1 - b0) * T)
        i_kv.append(add_copy(ckv_hbm.at[sl], ckv_v.at[sl]))
    i_uv = add_copy(wuv_hbm, wuv_v)
    i_o = add_copy(wo_hbm, wo_v)
    i_g = add_copy(wg_hbm, wg_v)
    i_u = add_copy(wu_hbm, wu_v)
    i_d = []
    for r0, r1 in WD_MXU + WD_VPU:
        sl = pl.ds(r0, r1 - r0)
        i_d.append(add_copy(wd_hbm.at[sl], wd_v.at[sl]))
    assert len(copies) == N_COPIES
    for i in range(N_COPIES):
        cp(i).start()

    ri = lax.broadcasted_iota(jnp.int32, (128, GW), 0)
    cj = lax.broadcasted_iota(jnp.int32, (128, GW), 1)
    e0 = jnp.where((cj // H) == ri, 1.0, 0.0).astype(BF16)
    hr = lax.broadcasted_iota(jnp.int32, (H, GW), 0)
    hc = lax.broadcasted_iota(jnp.int32, (H, GW), 1)
    diag = (hc % H) == hr

    def expand_mm(a, w_ref):
        a = a.astype(BF16)
        a_st = jnp.concatenate([a[:, g * 128:(g + 1) * 128] for g in range(G)], axis=0)
        xx = _dot(a_st, e0)
        out = None
        for g in range(G):
            s = jnp.where(diag, xx[g * H:(g + 1) * H], 0.0).astype(BF16)
            r = _dot(s, w_ref[pl.ds(g * GW, GW), :])
            out = r if out is None else out + r
        return out

    def contract_mm(q, w_ref, scale):
        q = q.astype(BF16)
        parts = []
        for g in range(G):
            tt = _dot_nt(q, w_ref[pl.ds(g * GW, GW), :])
            parts.append(jnp.where(diag, tt * scale, 0.0).astype(BF16))
        st = jnp.concatenate(parts, axis=0)
        r = _dot_nt(st, e0)
        return jnp.concatenate([r[g * H:(g + 1) * H] for g in range(G)], axis=1)

    cp(i_mod).wait()
    cp(i_c).wait()
    cp(i_x).wait()
    cc = jnp.broadcast_to(c_v[...].astype(F32), (8, M))
    sc = (cc * jax.nn.sigmoid(cc)).astype(BF16)
    mod = _dot(sc, wmod_v[...])
    sa, ca, ga, sb, cb, gb = [mod[:, i * M:(i + 1) * M] for i in range(6)]
    x = jnp.broadcast_to(x_v[0].astype(F32), (8, M))
    h = _layernorm(x) * (1.0 + ca) + sa

    cp(i_q).wait()
    hb = jnp.broadcast_to(h[0:1], (H, M))
    q = expand_mm(hb, wq_v)
    cp(i_uk).wait()
    qa = contract_mm(q, wuk_v, float(D) ** -0.5).astype(BF16)

    m_sc[...] = jnp.full((H, 128), -jnp.inf, F32)
    l_sc[...] = jnp.zeros((H, 128), F32)
    acc_sc[...] = jnp.zeros((H, DC), F32)

    def attn_step(i, carry):
        for j, (b0, _) in enumerate(KV_CHUNKS):
            @pl.when(i == b0)
            def _():
                cp(i_kv[j]).wait()

        kv = ckv_v[pl.ds(pl.multiple_of(i * T, T), T), :]
        s = _dot_nt(qa, kv)
        m_old = m_sc[...]
        m_new = jnp.maximum(m_old, jnp.max(s, axis=1, keepdims=True))
        alpha = jnp.exp(m_old - m_new)
        p = jnp.exp(s - m_new[:, 0:1])
        l_sc[...] = alpha * l_sc[...] + jnp.sum(p, axis=1, keepdims=True)
        m_sc[...] = m_new
        acc_sc[...] = alpha[:, 0:1] * acc_sc[...] + _dot(p.astype(BF16), kv)
        return carry

    lax.fori_loop(0, NKV, attn_step, 0)
    ctx_c = acc_sc[...] / l_sc[:, 0:1]

    cp(i_uv).wait()
    ctx = expand_mm(ctx_c, wuv_v).astype(BF16)
    cp(i_o).wait()
    row = lax.broadcasted_iota(jnp.int32, (H, D), 0)
    zero = jnp.zeros((H, D), BF16)
    lhs = jnp.concatenate([jnp.where(row == hh, ctx, zero) for hh in range(H)], axis=1)
    ao = jnp.sum(_dot(lhs, wo_v[...]), axis=0, keepdims=True)
    x2 = x + ga * ao

    h2 = (_layernorm(x2) * (1.0 + cb) + sb).astype(BF16)
    cp(i_g).wait()
    g = _dot(h2, wg_v[...])
    cp(i_u).wait()
    u = _dot(h2, wu_v[...])
    act = (jax.nn.gelu(g, approximate=True) * u).astype(BF16)
    for j in range(NL):
        act_sc[j] = act[:, j * FT:(j + 1) * FT]
    for t in range((DF - R0) // 128):
        a_t = jnp.transpose(act[:, R0 + t * 128:R0 + (t + 1) * 128].astype(F32))
        acol_sc[t * 128:(t + 1) * 128, :] = jnp.broadcast_to(a_t[:, 0:1], (128, 128))

    def down_step(j, y):
        for n, (r0, _) in enumerate(WD_MXU):
            @pl.when(j == r0 // FT)
            def _():
                cp(i_d[n]).wait()

        wd = wd_v[pl.ds(pl.multiple_of(j * FT, FT), FT), :]
        return y + _dot(act_sc[j], wd)

    y = lax.fori_loop(0, NL, down_step, jnp.zeros((8, M), F32))

    yv = None
    for n, (r0, r1) in enumerate(WD_VPU):
        acol = acol_sc[r0 - R0:r1 - R0, :]
        cp(i_d[len(WD_MXU) + n]).wait()
        w = wd_v[r0:r1, :].astype(F32)
        parts = []
        for t in range(M // 128):
            pr = w[:, t * 128:(t + 1) * 128] * acol
            a = pr[0:8]
            for k in range(1, (r1 - r0) // 8):
                a = a + pr[k * 8:(k + 1) * 8]
            parts.append(a)
        yb = jnp.concatenate(parts, axis=1)
        yv = yb if yv is None else yv + yb
    yv = jnp.sum(yv, axis=0, keepdims=True)
    out = x2[0:1] + gb[0:1] * (y[0:1] + yv)
    o_ref[0] = out.astype(o_ref.dtype)


@jax.jit
def pallas_adaLN_cond__compressed_kv_cla__glu_gated_geglu__decode_kernel(
    A_x: jax.Array,
    A_c_kv: jax.Array,
    A_w_q: jax.Array,
    A_w_uk: jax.Array,
    A_w_uv: jax.Array,
    A_w_o: jax.Array,
    B_x: jax.Array,
    B_w_gate: jax.Array,
    B_w_up: jax.Array,
    B_w_down: jax.Array,
    c: jax.Array,
    w_mod: jax.Array,
):
    del B_x
    M, H, D = A_w_q.shape
    DC = A_w_uk.shape[0]
    SK = A_c_kv.shape[1]
    DF = B_w_gate.shape[1]
    assert WD_VPU[-1][1] == DF

    ckv = A_c_kv.reshape(SK, DC)
    wq = A_w_q.reshape(M * H, D)
    wuk = A_w_uk.reshape(DC * H, D)
    wuv = A_w_uv.reshape(DC * H, D)
    wo = A_w_o.reshape(H * D, M)

    kern = functools.partial(_kernel, H=H, D=D, M=M, DC=DC, SK=SK, DF=DF)
    any_spec = pl.BlockSpec(memory_space=pl.ANY)
    return pl.pallas_call(
        kern,
        out_shape=jax.ShapeDtypeStruct(A_x.shape, A_x.dtype),
        in_specs=[any_spec] * 11,
        out_specs=pl.BlockSpec(memory_space=pltpu.VMEM),
        scratch_shapes=[
            pltpu.VMEM(A_x.shape, A_x.dtype),
            pltpu.VMEM(c.shape, c.dtype),
            pltpu.VMEM((SK, DC), BF16),
            pltpu.VMEM((M * H, D), BF16),
            pltpu.VMEM((DC * H, D), BF16),
            pltpu.VMEM((DC * H, D), BF16),
            pltpu.VMEM((H * D, M), BF16),
            pltpu.VMEM((M, DF), BF16),
            pltpu.VMEM((M, DF), BF16),
            pltpu.VMEM((DF, M), BF16),
            pltpu.VMEM(w_mod.shape, BF16),
            pltpu.VMEM((H, 128), F32),
            pltpu.VMEM((H, 128), F32),
            pltpu.VMEM((H, DC), F32),
            pltpu.VMEM((WD_MXU[-1][1] // FT, 8, FT), BF16),
            pltpu.VMEM((DF - WD_MXU[-1][1], 128), F32),
            pltpu.SemaphoreType.DMA((N_COPIES,)),
        ],
        compiler_params=pltpu.CompilerParams(vmem_limit_bytes=100 * 1024 * 1024,
                                             disable_semaphore_checks=True),
    )(A_x, ckv, wq, wuk, wuv, wo, B_w_gate, B_w_up, B_w_down, c, w_mod)
```
